```python
import os as _os
_os.environ.setdefault("JAX_PLATFORMS", "cpu")
import jax
import jax.numpy as jnp

def _softmax(x, axis=-1):
    return jax.nn.softmax(x, axis=axis)
def _gelu(x):
    return jax.nn.gelu(x, approximate=True)
def _silu(x):
    return jax.nn.silu(x)
def _sigmoid(x):
    return jax.nn.sigmoid(x)
def _layernorm(x, axis=-1, eps=1e-5):
    m = jnp.mean(x, axis=axis, keepdims=True)
    v = jnp.var(x, axis=axis, keepdims=True)
    return (x - m) / jnp.sqrt(v + eps)
def _scatter_add(tgt, idx, src, axis=0):
    return tgt.at[idx].add(src)
def _segment_sum(src, seg, n):
    return jax.ops.segment_sum(src, seg, n)
class _Rng:
    def __init__(self, key):
        self._k = key
    def _next(self):
        self._k, sub = jax.random.split(self._k)
        return sub
    def normal(self, shape):
        return jax.random.normal(self._next(), shape, dtype=jnp.bfloat16)
    def randint(self, lo, hi, shape):
        return jax.random.randint(self._next(), shape, lo, hi, dtype=jnp.int32)
    def uniform(self, shape, lo=0.0, hi=1.0):
        return jax.random.uniform(self._next(), shape, jnp.bfloat16, lo, hi)
    def permutation(self, n):
        return jax.random.permutation(self._next(), n)


kernel_name = 'standalone__gqa_softmax__decode'

def setup_inputs():
    _rng = _Rng(jax.random.key(int.from_bytes(__import__("os").urandom(4), "little")))
    _w = (lambda a: (lambda t: t.astype(jnp.bfloat16) if jnp.issubdtype(t.dtype, jnp.floating) else t)(jnp.asarray(a)))
    B, Hq, Hkv, Sq, Sk, D = 2, 32, 32, 1, 8192, 128
    return {
        "q": _w((lambda *s: _rng.normal(s) * 0.8)(B, Hq, Sq, D)),
        "k": _w((lambda *s: _rng.normal(s) * 0.8)(B, Hkv, Sk, D)),
        "v": _w((lambda *s: _rng.normal(s) * 0.05)(B, Hkv, Sk, D)),
    }

def reference(q, k, v):
    B, Hq, Sq, D = q.shape
    Hkv = k.shape[1]
    rep = Hq // Hkv
    k = jnp.repeat(k, rep, axis=1)
    v = jnp.repeat(v, rep, axis=1)
    scale = D ** -0.5
    scores = jnp.einsum("bhqd,bhkd->bhqk", q, k) * scale
    p = _softmax(scores, axis=-1)
    return jnp.einsum("bhqk,bhkd->bhqd", p, v)
```

```python
import math

import jax
import jax.numpy as jnp
from jax import lax
import jax.experimental.pallas as pl
import jax.experimental.pallas.tpu as pltpu

T = 128
G = 8
HS = 4
L = 16
NS = L + 1


@jax.jit
def pallas_standalone__gqa_softmax__decode_kernel(
    q: jax.Array,
    k: jax.Array,
    v: jax.Array,
):
    B, H, _, D = q.shape
    S = k.shape[2]
    NH = B * H
    NC = S // T
    NG = NH // G
    NSTEP = NG * NC
    c2 = (D ** -0.5) * math.log2(math.e)

    def head0(g):
        return lax.div(g, HS) * (HS * G) + lax.rem(g, HS)

    def row0(i):
        return head0(lax.div(i, NC)) * S + lax.rem(i, NC) * T

    def kernel(q_hbm, k_hbm, v_hbm, o_hbm, buf, qv, q32, sc, o32, ov, sems, qsem, osem):
        def start_tile(src, r0, slot, j):
            r = r0 + j * HS * S
            if not isinstance(r, int):
                r = pl.multiple_of(r, T)
            pltpu.make_async_copy(
                src.at[pl.ds(r, T)], buf.at[slot, j], sems.at[slot]
            ).start(priority=j % 2)

        def wait(slot):
            pltpu.make_async_copy(buf.at[slot], buf.at[slot], sems.at[slot]).wait()

        def nxt(slot):
            return jnp.where(slot == NS - 1, 0, slot + 1)

        for j in range(G):
            start_tile(k_hbm, 0, 0, j)
        qc = pltpu.make_async_copy(q_hbm, qv, qsem)
        qc.start()

        def prologue(i, _):
            r0 = row0(i)
            for j in range(G):
                start_tile(k_hbm, r0, i, j)

        lax.fori_loop(1, L, prologue, None)
        qc.wait()
        q32[...] = qv[...].astype(jnp.float32)

        row = lax.broadcasted_iota(jnp.int32, (G, D), 0)

        def qk_group(g, slots, last):
            q8 = q32[pl.ds(head0(g), G, stride=HS), :].astype(jnp.bfloat16)

            def body(src, shift):
                def step(c, carry):
                    mx, slot, wslot = carry
                    i = g * NC + c
                    wait(slot)
                    r0 = row0(i + shift)
                    s = None
                    for j in range(G):
                        kt = buf[slot, j]
                        start_tile(src, r0, wslot, j)
                        r = lax.dot_general(
                            q8, kt, (((1,), (1,)), ((), ())),
                            preferred_element_type=jnp.float32)
                        s = r if s is None else jnp.where(row == j, r, s)
                    sc[i] = s
                    return jnp.maximum(mx, s), nxt(slot), nxt(wslot)
                return step

            carry = (jnp.full((G, T), -jnp.inf, jnp.float32),) + slots
            if last:
                carry = lax.fori_loop(0, NC - L, body(k_hbm, L), carry)
                carry = lax.fori_loop(NC - L, NC, body(v_hbm, L - NSTEP), carry)
            else:
                carry = lax.fori_loop(0, NC, body(k_hbm, L), carry)
            mx = jnp.max(carry[0], axis=1, keepdims=True)
            sc[NSTEP + g] = jnp.broadcast_to(mx, (G, T))
            return carry[1:]

        slots = (jnp.int32(0), jnp.int32(L % NS))
        slots = lax.fori_loop(0, NG - 1, lambda g, s: qk_group(g, s, False), slots)
        slots = qk_group(jnp.int32(NG - 1), slots, True)

        def pv_group(g, slots, last):
            m = sc[NSTEP + g]

            def body(src):
                def step(c, carry):
                    l, accs, slot, wslot = carry
                    i = g * NC + c
                    p = jnp.exp2((sc[i] - m) * c2)
                    pb = p.astype(jnp.bfloat16)
                    wait(slot)
                    r0 = row0(i + L) if src is not None else None
                    out = []
                    for j in range(G):
                        vt = buf[slot, j]
                        if src is not None:
                            start_tile(src, r0, wslot, j)
                        out.append(accs[j] + jnp.dot(pb, vt, preferred_element_type=jnp.float32))
                    return l + p, tuple(out), nxt(slot), nxt(wslot)
                return step

            z = jnp.zeros((G, D), jnp.float32)
            carry = (z, (z,) * G) + slots
            if last:
                carry = lax.fori_loop(0, NC - L, body(v_hbm), carry)
                carry = lax.fori_loop(NC - L, NC, body(None), carry)
            else:
                carry = lax.fori_loop(0, NC, body(v_hbm), carry)
            l, accs = carry[:2]
            acc = accs[0]
            for j in range(1, G):
                acc = jnp.where(row == j, accs[j], acc)
            o32[pl.ds(head0(g), G, stride=HS), :] = acc / jnp.sum(l, axis=1, keepdims=True)
            return carry[2:]

        slots = lax.fori_loop(0, NG - 1, lambda g, s: pv_group(g, s, False), slots)
        pv_group(jnp.int32(NG - 1), slots, True)

        ov[...] = o32[...].astype(ov.dtype)
        oc = pltpu.make_async_copy(ov, o_hbm, osem)
        oc.start()
        oc.wait()

    o = pl.pallas_call(
        kernel,
        out_shape=jax.ShapeDtypeStruct((NH, D), q.dtype),
        in_specs=[pl.BlockSpec(memory_space=pl.ANY)] * 3,
        out_specs=pl.BlockSpec(memory_space=pl.ANY),
        scratch_shapes=[
            pltpu.VMEM((NS, G, T, D), k.dtype),
            pltpu.VMEM((NH, D), q.dtype),
            pltpu.VMEM((NH, D), jnp.float32),
            pltpu.VMEM((NSTEP + NG, G, T), jnp.float32),
            pltpu.VMEM((NH, D), jnp.float32),
            pltpu.VMEM((NH, D), q.dtype),
            pltpu.SemaphoreType.DMA((NS,)),
            pltpu.SemaphoreType.DMA(()),
            pltpu.SemaphoreType.DMA(()),
        ],
        compiler_params=pltpu.CompilerParams(
            disable_semaphore_checks=True,
            disable_bounds_checks=True,
        ),
        name="gqa_decode",
    )(q.reshape(NH, D), k.reshape(NH * S, D), v.reshape(NH * S, D))
    return o.reshape(B, H, 1, D)
```

```python
import math

import jax
import jax.numpy as jnp
from jax import lax
import jax.experimental.pallas as pl
import jax.experimental.pallas.tpu as pltpu

T = 128
G = 8
P = 2
HALF = 64
L = 8
NS = L + 1
COPIES = tuple(
    (4 * (n & 1) + 2 * ((n >> 2) & 1), (n >> 1) & 1, HALF * (n >> 3)) for n in range(16)
)


@jax.jit
def pallas_standalone__gqa_softmax__decode_kernel(
    q: jax.Array,
    k: jax.Array,
    v: jax.Array,
):
    B, H, _, D = q.shape
    S = k.shape[2]
    NH = B * H
    NC = S // (P * T)
    NG = NH // G
    NSTEP = NG * NC
    c2 = (D ** -0.5) * math.log2(math.e)
    tiles = [(a, j) for a in range(P) for j in range(G)]

    def kernel(q_hbm, k_hbm, v_hbm, o_hbm, buf, qv, q32, sc, o32, ov, sems, qsem, osem):
        def start(src, i, slot, n):
            h, a, r = COPIES[n]
            if isinstance(i, int):
                h0, r0 = (i // NC) * G + h, (i % NC) * T + r
            else:
                h0 = lax.div(i, NC) * G + h
                r0 = pl.multiple_of(lax.rem(i, NC) * T + r, HALF)
            pltpu.make_async_copy(
                src.at[pl.ds(h0, 2), pl.ds(a, 1), pl.ds(r0, HALF)],
                buf.at[slot, pl.ds(h, 2), pl.ds(a, 1), pl.ds(r, HALF)],
                sems.at[slot],
            ).start(priority=n % 2)

        def wait(slot):
            pltpu.make_async_copy(buf.at[slot], buf.at[slot], sems.at[slot]).wait()

        def nxt(slot):
            return jnp.where(slot == NS - 1, 0, slot + 1)

        for n in range(len(COPIES)):
            start(k_hbm, 0, 0, n)
        qc = pltpu.make_async_copy(q_hbm, qv, qsem)
        qc.start()

        def prologue(i, _):
            for n in range(len(COPIES)):
                start(k_hbm, i, i, n)

        lax.fori_loop(1, L, prologue, None)
        qc.wait()
        q32[...] = qv[...].astype(jnp.float32)

        row = lax.broadcasted_iota(jnp.int32, (G, D), 0)

        def qk_group(g, slots, last):
            q8 = q32[pl.ds(pl.multiple_of(g * G, G), G), :].astype(jnp.bfloat16)

            def body(src, shift):
                def step(c, carry):
                    mx, slot, wslot = carry
                    i = g * NC + c
                    wait(slot)
                    s = [None] * P
                    for n, (a, j) in enumerate(tiles):
                        kt = buf[slot, j, a]
                        start(src, i + shift, wslot, n)
                        x = lax.dot_general(
                            q8, kt, (((1,), (1,)), ((), ())),
                            preferred_element_type=jnp.float32)
                        s[a] = x if s[a] is None else jnp.where(row == j, x, s[a])
                    for a in range(P):
                        sc[i * P + a] = s[a]
                        mx = jnp.maximum(mx, s[a])
                    return mx, nxt(slot), nxt(wslot)
                return step

            carry = (jnp.full((G, T), -jnp.inf, jnp.float32),) + slots
            if last:
                carry = lax.fori_loop(0, NC - L, body(k_hbm, L), carry)
                carry = lax.fori_loop(NC - L, NC, body(v_hbm, L - NSTEP), carry)
            else:
                carry = lax.fori_loop(0, NC, body(k_hbm, L), carry)
            mx = jnp.max(carry[0], axis=1, keepdims=True)
            sc[NSTEP * P + g] = jnp.broadcast_to(mx, (G, T))
            return carry[1:]

        slots = (jnp.int32(0), jnp.int32(L % NS))
        slots = lax.fori_loop(0, NG - 1, lambda g, s: qk_group(g, s, False), slots)
        slots = qk_group(jnp.int32(NG - 1), slots, True)

        def pv_group(g, slots, last):
            m = sc[NSTEP * P + g]

            def body(src):
                def step(c, carry):
                    l, accs, slot, wslot = carry
                    i = g * NC + c
                    ps = [jnp.exp2((sc[i * P + a] - m) * c2) for a in range(P)]
                    pbs = [p.astype(jnp.bfloat16) for p in ps]
                    wait(slot)
                    accs = list(accs)
                    for n, (a, j) in enumerate(tiles):
                        vt = buf[slot, j, a]
                        if src is not None:
                            start(src, i + L, wslot, n)
                        accs[j] = accs[j] + jnp.dot(
                            pbs[a], vt, preferred_element_type=jnp.float32)
                    for p in ps:
                        l = l + p
                    return l, tuple(accs), nxt(slot), nxt(wslot)
                return step

            z = jnp.zeros((G, D), jnp.float32)
            carry = (z, (z,) * G) + slots
            if last:
                carry = lax.fori_loop(0, NC - L, body(v_hbm), carry)
                carry = lax.fori_loop(NC - L, NC, body(None), carry)
            else:
                carry = lax.fori_loop(0, NC, body(v_hbm), carry)
            l, accs = carry[:2]
            acc = accs[0]
            for j in range(1, G):
                acc = jnp.where(row == j, accs[j], acc)
            o32[pl.ds(pl.multiple_of(g * G, G), G), :] = acc / jnp.sum(l, axis=1, keepdims=True)
            return carry[2:]

        slots = lax.fori_loop(0, NG - 1, lambda g, s: pv_group(g, s, False), slots)
        pv_group(jnp.int32(NG - 1), slots, True)

        ov[...] = o32[...].astype(ov.dtype)
        oc = pltpu.make_async_copy(ov, o_hbm, osem)
        oc.start()
        oc.wait()

    o = pl.pallas_call(
        kernel,
        out_shape=jax.ShapeDtypeStruct((NH, D), q.dtype),
        in_specs=[pl.BlockSpec(memory_space=pl.ANY)] * 3,
        out_specs=pl.BlockSpec(memory_space=pl.ANY),
        scratch_shapes=[
            pltpu.VMEM((NS, G, P, T, D), k.dtype),
            pltpu.VMEM((NH, D), q.dtype),
            pltpu.VMEM((NH, D), jnp.float32),
            pltpu.VMEM((NSTEP * P + NG, G, T), jnp.float32),
            pltpu.VMEM((NH, D), jnp.float32),
            pltpu.VMEM((NH, D), q.dtype),
            pltpu.SemaphoreType.DMA((NS,)),
            pltpu.SemaphoreType.DMA(()),
            pltpu.SemaphoreType.DMA(()),
        ],
        compiler_params=pltpu.CompilerParams(
            disable_semaphore_checks=True,
            disable_bounds_checks=True,
        ),
        name="gqa_decode",
    )(q.reshape(NH, D), k.reshape(NH, P, S // P, D), v.reshape(NH, P, S // P, D))
    return o.reshape(B, H, 1, D)
```

```python
import math

import jax
import jax.numpy as jnp
from jax import lax
import jax.experimental.pallas as pl
import jax.experimental.pallas.tpu as pltpu

TILE = 128
HALF = TILE // 2
HEADS = 8
ORDER = (0, 4, 1, 5, 2, 6, 3, 7)
AHEAD = (5, 11)
SLOTS = 16


def _divmod(step, n):
    if isinstance(step, int):
        return divmod(step, n)
    return lax.div(step, n), lax.rem(step, n)


def _aligned(x, n):
    return x if isinstance(x, int) else pl.multiple_of(x, n)


def _loop(start, stop, body):
    lax.fori_loop(start, stop, lambda step, _: body(step), None)


def _own_rows(xs):
    sublane = lax.broadcasted_iota(jnp.int32, xs[0].shape, 0)
    x = xs[0]
    for n in range(1, HEADS):
        x = jnp.where(sublane == ORDER[n], xs[n], x)
    return x


def _kernel(q_hbm, k_hbm, v_hbm, o_hbm,
            ring, q_raw, q_f32, scores, row_max, denom, acc, out,
            ring_sems, q_sem, o_sem):
    heads, _, half_keys, d = k_hbm.shape
    per_group = half_keys // HALF
    steps = heads // HEADS * per_group
    near, far = AHEAD
    exp2_scale = d ** -0.5 * math.log2(math.e)

    def fetch(src, step, n):
        group, chunk = _divmod(step, per_group)
        slot = _divmod(step, SLOTS)[1]
        pltpu.make_async_copy(
            src.at[group * HEADS + ORDER[n], :, pl.ds(_aligned(chunk * HALF, HALF), HALF)],
            ring.at[slot, n],
            ring_sems.at[slot],
        ).start(priority=n % 2)

    def products(step, product, prefetch):
        slot = _divmod(step, SLOTS)[1]
        pltpu.make_async_copy(ring.at[slot], ring.at[slot], ring_sems.at[slot]).wait()
        xs = []
        for n in range(HEADS):
            tile = ring[slot, n].reshape(TILE, d)
            if prefetch[n % 2] is not None:
                src, offset = prefetch[n % 2]
                fetch(src, step + offset, n)
            xs.append(product(tile))
        return _own_rows(xs)

    def rows_of(step):
        return pl.ds(_aligned(_divmod(step, per_group)[0] * HEADS, HEADS), HEADS)

    for step in range(far - near):
        for n in range(1, HEADS, 2):
            fetch(k_hbm, step, n)
    q_copy = pltpu.make_async_copy(q_hbm, q_raw, q_sem)
    q_copy.start()

    def fill(step):
        for n in range(HEADS):
            fetch(k_hbm, step + (far - near) * (n % 2), n)

    _loop(0, near, fill)
    row_max[...] = jnp.full(row_max.shape, -jnp.inf, jnp.float32)
    denom[...] = jnp.zeros(denom.shape, jnp.float32)
    acc[...] = jnp.zeros(acc.shape, jnp.float32)
    q_copy.wait()
    q_f32[...] = q_raw[...].astype(jnp.float32)

    def score_step(prefetch):
        def body(step):
            rows = rows_of(step)
            q = q_f32[rows, :].astype(ring.dtype)
            s = products(
                step,
                lambda tile: lax.dot_general(
                    q, tile, (((1,), (1,)), ((), ())),
                    preferred_element_type=jnp.float32),
                prefetch)
            scores[step] = s
            row_max[rows, :] = jnp.maximum(row_max[rows, :], s)
        return body

    _loop(0, steps - far, score_step(((k_hbm, near), (k_hbm, far))))
    _loop(steps - far, steps - near, score_step(((k_hbm, near), (v_hbm, far - steps))))
    _loop(steps - near, steps, score_step(((v_hbm, near - steps), (v_hbm, far - steps))))
    row_max[...] = jnp.broadcast_to(
        jnp.max(row_max[...], axis=1, keepdims=True), row_max.shape)

    def weights(step):
        rows = rows_of(step)
        p = jnp.exp2((scores[step] - row_max[rows, :]) * exp2_scale)
        denom[rows, :] += p
        return p.astype(ring.dtype)

    def values(step, p, prefetch):
        return products(
            step,
            lambda tile: jnp.dot(p, tile, preferred_element_type=jnp.float32),
            prefetch)

    def value_step(prefetch):
        def body(step):
            x = values(step, weights(step), prefetch)
            acc[rows_of(step), :] += x
        return body

    _loop(0, steps - far, value_step(((v_hbm, near), (v_hbm, far))))
    _loop(steps - far, steps - near, value_step(((v_hbm, near), None)))
    _loop(steps - near, steps - 1, value_step((None, None)))

    p = weights(steps - 1)
    inv = 1.0 / jnp.sum(denom[...], axis=1, keepdims=True)
    done = heads - 2 * HEADS
    out[:done, :] = (acc[:done, :] * inv[:done]).astype(out.dtype)
    x = values(steps - 1, p, (None, None))
    rest = jnp.concatenate(
        [acc[done:heads - HEADS, :], acc[heads - HEADS:, :] + x], axis=0)
    out[done:, :] = (rest * inv[done:]).astype(out.dtype)
    o_copy = pltpu.make_async_copy(out, o_hbm, o_sem)
    o_copy.start()
    o_copy.wait()


@jax.jit
def pallas_standalone__gqa_softmax__decode_kernel(
    q: jax.Array,
    k: jax.Array,
    v: jax.Array,
):
    b, hq, sq, d = q.shape
    _, hkv, sk, _ = k.shape
    heads = b * hq
    steps = heads // HEADS * (sk // TILE)
    assert sq == 1 and hq == hkv, "one query per head, one KV head per query head"
    assert heads % (2 * HEADS) == 0 and heads > 2 * HEADS and sk % TILE == 0
    assert steps % SLOTS == 0, "both passes must start at ring slot 0"

    out = pl.pallas_call(
        _kernel,
        out_shape=jax.ShapeDtypeStruct((heads, d), q.dtype),
        in_specs=[pl.BlockSpec(memory_space=pl.ANY)] * 3,
        out_specs=pl.BlockSpec(memory_space=pl.ANY),
        scratch_shapes=[
            pltpu.VMEM((SLOTS, HEADS, 2, HALF, d), k.dtype),
            pltpu.VMEM((heads, d), q.dtype),
            pltpu.VMEM((heads, d), jnp.float32),
            pltpu.VMEM((steps, HEADS, TILE), jnp.float32),
            pltpu.VMEM((heads, TILE), jnp.float32),
            pltpu.VMEM((heads, TILE), jnp.float32),
            pltpu.VMEM((heads, d), jnp.float32),
            pltpu.VMEM((heads, d), q.dtype),
            pltpu.SemaphoreType.DMA((SLOTS,)),
            pltpu.SemaphoreType.DMA(()),
            pltpu.SemaphoreType.DMA(()),
        ],
        compiler_params=pltpu.CompilerParams(
            disable_bounds_checks=True,
            disable_semaphore_checks=True,
        ),
        name="gqa_decode",
    )(
        q.reshape(heads, d),
        k.reshape(heads, 2, sk // 2, d),
        v.reshape(heads, 2, sk // 2, d),
    )
    return out.reshape(q.shape)
```
